```python
import os as _os
_os.environ.setdefault("JAX_PLATFORMS", "cpu")
import jax
import jax.numpy as jnp

def _softmax(x, axis=-1):
    return jax.nn.softmax(x, axis=axis)
def _gelu(x):
    return jax.nn.gelu(x, approximate=True)
def _silu(x):
    return jax.nn.silu(x)
def _sigmoid(x):
    return jax.nn.sigmoid(x)
def _layernorm(x, axis=-1, eps=1e-5):
    m = jnp.mean(x, axis=axis, keepdims=True)
    v = jnp.var(x, axis=axis, keepdims=True)
    return (x - m) / jnp.sqrt(v + eps)
def _scatter_add(tgt, idx, src, axis=0):
    return tgt.at[idx].add(src)
def _segment_sum(src, seg, n):
    return jax.ops.segment_sum(src, seg, n)
class _Rng:
    def __init__(self, key):
        self._k = key
    def _next(self):
        self._k, sub = jax.random.split(self._k)
        return sub
    def normal(self, shape):
        return jax.random.normal(self._next(), shape, dtype=jnp.bfloat16)
    def randint(self, lo, hi, shape):
        return jax.random.randint(self._next(), shape, lo, hi, dtype=jnp.int32)
    def uniform(self, shape, lo=0.0, hi=1.0):
        return jax.random.uniform(self._next(), shape, jnp.bfloat16, lo, hi)
    def permutation(self, n):
        return jax.random.permutation(self._next(), n)


kernel_name = 'standalone__gqa_softmax__near_ridge'

def setup_inputs():
    _rng = _Rng(jax.random.key(int.from_bytes(__import__("os").urandom(4), "little")))
    _w = (lambda a: (lambda t: t.astype(jnp.bfloat16) if jnp.issubdtype(t.dtype, jnp.floating) else t)(jnp.asarray(a)))
    B, Hq, Hkv, Sq, Sk, D = 8, 16, 8, 160, 2048, 256
    return {
        "q": _w((lambda *s: _rng.normal(s) * 0.05)(B, Hq, Sq, D)),
        "k": _w((lambda *s: _rng.normal(s) * 3.2)(B, Hkv, Sk, D)),
        "v": _w((lambda *s: _rng.normal(s) * 0.05)(B, Hkv, Sk, D)),
    }

def reference(q, k, v):
    B, Hq, Sq, D = q.shape
    Hkv = k.shape[1]
    rep = Hq // Hkv
    k = jnp.repeat(k, rep, axis=1)
    v = jnp.repeat(v, rep, axis=1)
    scale = D ** -0.5
    scores = jnp.einsum("bhqd,bhkd->bhqk", q, k) * scale
    p = _softmax(scores, axis=-1)
    return jnp.einsum("bhqk,bhkd->bhqd", p, v)
```

```python
import functools

import jax
import jax.numpy as jnp
import jax.experimental.pallas as pl
import jax.experimental.pallas.tpu as pltpu
from jax import lax

_LOG2E = 1.4426950408889634
_LANES = 128
_CHUNK = 512
_NBUF = 4
_NOUT = 4
_UNROLL = 4


def _fold(x, op):
    out = x[:, 0:_LANES]
    for j in range(1, x.shape[1] // _LANES):
        out = op(out, x[:, j * _LANES:(j + 1) * _LANES])
    return out


def _rep(x, n):
    return jnp.concatenate([x] * n, axis=1) if n > 1 else x


def _attention_kernel(q_hbm, k_hbm, v_hbm, o_hbm,
                      qbuf, kbuf, vbuf, obuf, m_ref, l0, l1, acc0, acc1, isem, osem,
                      *, scale, ng, rows, sk, d, chunk, unroll):
    c = scale * _LOG2E
    nr = sk // chunk
    l_refs = (l0, l1)
    acc_refs = (acc0, acc1)

    def in_copies(g, r):
        slot = g % _NBUF
        sem = isem.at[slot, r]
        keys = pl.ds(r * chunk, chunk)
        copies = [pltpu.make_async_copy(k_hbm.at[g, keys], kbuf.at[slot, keys], sem),
                  pltpu.make_async_copy(v_hbm.at[g, keys], vbuf.at[slot, keys], sem)]
        if r == 0:
            copies.insert(0, pltpu.make_async_copy(q_hbm.at[g], qbuf.at[slot], sem))
        return copies

    def start_in(g, r):
        for cp in in_copies(g, r):
            cp.start()

    def wait_in(g, r):
        for cp in in_copies(g, r):
            cp.wait()

    def out_copy(g):
        slot = g % _NOUT
        return pltpu.make_async_copy(obuf.at[slot], o_hbm.at[g], osem.at[slot])

    def finalize(g, par):
        l = jnp.sum(l_refs[par][...], axis=-1, keepdims=True)
        obuf[g % _NOUT] = (acc_refs[par][...] * (1.0 / l)).astype(obuf.dtype)

    def step(i, par, first):
        slot = i % _NBUF
        for r in range(nr):
            q = qbuf[slot]
            k = kbuf[slot, pl.ds(r * chunk, chunk), :]
            s = lax.dot_general(q, k, (((1,), (1,)), ((), ())),
                                preferred_element_type=jnp.float32)

            if r == 0:
                if first:
                    @pl.when(i == 0)
                    def _():
                        for g in range(2, _NBUF - 1):
                            for rr in range(nr):
                                start_in(g, rr)

                @pl.when(i + _NBUF - 1 < ng)
                def _():
                    for rr in range(nr):
                        start_in(i + _NBUF - 1, rr)

                @pl.when(i >= 2)
                def _():
                    out_copy(i - 2).start()

            if r == min(1, nr - 1):
                @pl.when(i > _NOUT)
                def _():
                    out_copy(i - 1 - _NOUT).wait()
                finalize(i - 1, 1 - par)

            m_blk = jnp.max(_fold(s, jnp.maximum), axis=-1, keepdims=True)
            m_blk = jnp.broadcast_to(m_blk, (rows, _LANES))
            if r == 0:
                m_new = m_blk
            else:
                m_old = m_ref[...]
                m_new = jnp.maximum(m_old, m_blk)
                alpha = jnp.exp2((m_old - m_new) * c)
            if r < nr - 1:
                m_ref[...] = m_new
            p = jnp.exp2((s - _rep(m_new, chunk // _LANES)) * c)
            l_blk = _fold(p, jnp.add)
            l_refs[par][...] = l_blk if r == 0 else l_refs[par][...] * alpha + l_blk

            if r + 1 < nr:
                wait_in(i, r + 1)
            else:
                @pl.when(i + 1 < ng)
                def _():
                    wait_in(i + 1, 0)

            v = vbuf[slot, pl.ds(r * chunk, chunk), :]
            o = jnp.dot(p.astype(v.dtype), v, preferred_element_type=jnp.float32)
            acc_refs[par][...] = o if r == 0 else (
                acc_refs[par][...] * _rep(alpha, d // _LANES) + o)

    for r in range(nr):
        start_in(0, r)
    l1[...] = jnp.ones(l1.shape, l1.dtype)
    acc1[...] = jnp.zeros(acc1.shape, acc1.dtype)
    wait_in(0, 0)
    for r in range(nr):
        start_in(1, r)

    def body(it, carry):
        for u in range(unroll):
            step(it * unroll + u, u % 2, u == 0)
        return carry

    lax.fori_loop(0, ng // unroll, body, 0)

    out_copy(ng - 1 - _NOUT).wait()
    out_copy(ng - 2).start()
    finalize(ng - 1, (ng - 1) % 2)
    out_copy(ng - 1).start()
    for g in range(ng - _NOUT, ng):
        out_copy(g).wait()


@jax.jit
def pallas_standalone__gqa_softmax__near_ridge_kernel(
    q: jax.Array,
    k: jax.Array,
    v: jax.Array,
):
    b, hq, sq, d = q.shape
    _, hkv, sk, _ = k.shape
    rows = (hq // hkv) * sq
    ng = b * hkv
    chunk = min(_CHUNK, sk)
    assert hq % hkv == 0 and sk % chunk == 0 and chunk % _LANES == 0 and d % _LANES == 0
    assert ng % _UNROLL == 0 and ng >= 2 * _NOUT and rows % 16 == 0

    out = pl.pallas_call(
        functools.partial(_attention_kernel, scale=d ** -0.5, ng=ng, rows=rows, sk=sk,
                          d=d, chunk=chunk, unroll=_UNROLL),
        in_specs=[pl.BlockSpec(memory_space=pl.ANY)] * 3,
        out_specs=pl.BlockSpec(memory_space=pl.ANY),
        out_shape=jax.ShapeDtypeStruct((ng, rows, d), q.dtype),
        scratch_shapes=[
            pltpu.VMEM((_NBUF, rows, d), q.dtype),
            pltpu.VMEM((_NBUF, sk, d), k.dtype),
            pltpu.VMEM((_NBUF, sk, d), v.dtype),
            pltpu.VMEM((_NOUT, rows, d), q.dtype),
            pltpu.VMEM((rows, _LANES), jnp.float32),
            pltpu.VMEM((rows, _LANES), jnp.float32),
            pltpu.VMEM((rows, _LANES), jnp.float32),
            pltpu.VMEM((rows, d), jnp.float32),
            pltpu.VMEM((rows, d), jnp.float32),
            pltpu.SemaphoreType.DMA((_NBUF, sk // chunk)),
            pltpu.SemaphoreType.DMA((_NOUT,)),
        ],
        compiler_params=pltpu.CompilerParams(
            vmem_limit_bytes=64 * 1024 * 1024,
            disable_bounds_checks=True,
            flags={"XLA_TPU_RESCHEDULE_DMA_DONES": True},
        ),
    )(q.reshape(ng, rows, d), k.reshape(ng, sk, d), v.reshape(ng, sk, d))
    return out.reshape(b, hq, sq, d)
```

```python
import functools

import jax
import jax.numpy as jnp
import jax.experimental.pallas as pl
import jax.experimental.pallas.tpu as pltpu
from jax import lax

_LOG2E = 1.4426950408889634
_LANES = 128
_CHUNK = 512
_RING = 4

_reciprocal = pltpu.reciprocal if hasattr(pltpu, "reciprocal") else pl.reciprocal


def _fold(x, op):
    out = x[:, 0:_LANES]
    for j in range(1, x.shape[1] // _LANES):
        out = op(out, x[:, j * _LANES:(j + 1) * _LANES])
    return out


def _rep(x, n):
    return jnp.concatenate([x] * n, axis=1) if n > 1 else x


def _attention_kernel(q_hbm, k_hbm, v_hbm, o_hbm,
                      qbuf, kbuf, vbuf, obuf, m_ref, l0, l1, acc0, acc1, isem, osem,
                      *, scale, ng, rows, sk, d, chunk):
    c = scale * _LOG2E
    nr = sk // chunk
    l_refs = (l0, l1)
    acc_refs = (acc0, acc1)

    def in_copies(g, slot, sec):
        sem = isem.at[slot, sec]
        copies = []
        if sec == 0:
            copies.append(pltpu.make_async_copy(q_hbm.at[g], qbuf.at[slot], sem))
        if sec < nr:
            keys = pl.ds(sec * chunk, chunk)
            copies.append(pltpu.make_async_copy(k_hbm.at[g, keys], kbuf.at[slot, keys], sem))
        if sec > 0:
            keys = pl.ds((sec - 1) * chunk, chunk)
            copies.append(pltpu.make_async_copy(v_hbm.at[g, keys], vbuf.at[slot, keys], sem))
        return copies

    def start_group(g, slot):
        for sec in range(nr + 1):
            for cp in in_copies(g, slot, sec):
                cp.start()

    def wait_in(g, slot, sec):
        for cp in in_copies(g, slot, sec):
            cp.wait()

    def out_copy(g, slot):
        return pltpu.make_async_copy(obuf.at[slot], o_hbm.at[g], osem.at[slot])

    def finalize(slot):
        par = slot % 2
        l = jnp.sum(l_refs[par][...], axis=-1, keepdims=True)
        inv = _reciprocal(l, approx=True)
        inv = inv + inv * (1.0 - l * inv)
        obuf[slot] = (acc_refs[par][...] * inv).astype(obuf.dtype)

    def step(i, slot):
        par = slot % 2
        prev, prev2, nxt = (slot - 1) % _RING, (slot - 2) % _RING, (slot + 1) % _RING
        for r in range(nr):
            q = qbuf[slot]
            k = kbuf[slot, pl.ds(r * chunk, chunk), :]
            s = lax.dot_general(q, k, (((1,), (1,)), ((), ())),
                                preferred_element_type=jnp.float32)

            if r == 0:
                if slot == 0:
                    @pl.when(i == 0)
                    def _():
                        for g in range(2, _RING - 1):
                            start_group(g, g)

                @pl.when(i + _RING - 1 < ng)
                def _():
                    start_group(i + _RING - 1, prev)

                @pl.when(i >= 2)
                def _():
                    out_copy(i - 2, prev2).start()

            if r == min(1, nr - 1):
                @pl.when(i > _RING)
                def _():
                    out_copy(i - 1 - _RING, prev).wait()
                finalize(prev)

            m_blk = jnp.max(_fold(s, jnp.maximum), axis=-1, keepdims=True)
            m_blk = jnp.broadcast_to(m_blk, (rows, _LANES)) * c
            if r == 0:
                m_new = m_blk
            else:
                m_old = m_ref[...]
                m_new = jnp.maximum(m_old, m_blk)
                alpha = jnp.exp2(m_old - m_new)
            if r < nr - 1:
                m_ref[...] = m_new
            p = jnp.exp2(s * c - _rep(m_new, chunk // _LANES))
            l_blk = _fold(p, jnp.add)
            l_refs[par][...] = l_blk if r == 0 else l_refs[par][...] * alpha + l_blk

            wait_in(i, slot, r + 1)
            if r == nr - 1:
                @pl.when(i + 1 < ng)
                def _():
                    wait_in(i + 1, nxt, 0)

            v = vbuf[slot, pl.ds(r * chunk, chunk), :]
            o = jnp.dot(p.astype(v.dtype), v, preferred_element_type=jnp.float32)
            acc_refs[par][...] = o if r == 0 else (
                acc_refs[par][...] * _rep(alpha, d // _LANES) + o)

    start_group(0, 0)
    l1[...] = jnp.ones(l1.shape, l1.dtype)
    acc1[...] = jnp.zeros(acc1.shape, acc1.dtype)
    wait_in(0, 0, 0)
    start_group(1, 1)

    def body(it, carry):
        for u in range(_RING):
            step(it * _RING + u, u)
        return carry

    lax.fori_loop(0, ng // _RING, body, 0)

    last = _RING - 1
    out_copy(ng - 1 - _RING, last).wait()
    out_copy(ng - 2, last - 1).start()
    finalize(last)
    out_copy(ng - 1, last).start()
    for g in range(ng - _RING, ng):
        out_copy(g, g % _RING).wait()


@jax.jit
def pallas_standalone__gqa_softmax__near_ridge_kernel(
    q: jax.Array,
    k: jax.Array,
    v: jax.Array,
):
    b, hq, sq, d = q.shape
    _, hkv, sk, _ = k.shape
    rows = (hq // hkv) * sq
    ng = b * hkv
    chunk = min(_CHUNK, sk)
    assert hq % hkv == 0 and sk % chunk == 0 and chunk % _LANES == 0 and d % _LANES == 0
    assert ng % _RING == 0 and ng >= 2 * _RING and rows % 16 == 0

    out = pl.pallas_call(
        functools.partial(_attention_kernel, scale=d ** -0.5, ng=ng, rows=rows, sk=sk,
                          d=d, chunk=chunk),
        in_specs=[pl.BlockSpec(memory_space=pl.ANY)] * 3,
        out_specs=pl.BlockSpec(memory_space=pl.ANY),
        out_shape=jax.ShapeDtypeStruct((ng, rows, d), q.dtype),
        scratch_shapes=[
            pltpu.VMEM((_RING, rows, d), q.dtype),
            pltpu.VMEM((_RING, sk, d), k.dtype),
            pltpu.VMEM((_RING, sk, d), v.dtype),
            pltpu.VMEM((_RING, rows, d), q.dtype),
            pltpu.VMEM((rows, _LANES), jnp.float32),
            pltpu.VMEM((rows, _LANES), jnp.float32),
            pltpu.VMEM((rows, _LANES), jnp.float32),
            pltpu.VMEM((rows, d), jnp.float32),
            pltpu.VMEM((rows, d), jnp.float32),
            pltpu.SemaphoreType.DMA((_RING, sk // chunk + 1)),
            pltpu.SemaphoreType.DMA((_RING,)),
        ],
        compiler_params=pltpu.CompilerParams(
            vmem_limit_bytes=64 * 1024 * 1024,
            disable_bounds_checks=True,
            flags={"XLA_TPU_RESCHEDULE_DMA_DONES": True},
        ),
    )(q.reshape(ng, rows, d), k.reshape(ng, sk, d), v.reshape(ng, sk, d))
    return out.reshape(b, hq, sq, d)
```
